```python
import os as _os
_os.environ.setdefault("JAX_PLATFORMS", "cpu")
import jax
import jax.numpy as jnp

def _softmax(x, axis=-1):
    return jax.nn.softmax(x, axis=axis)
def _gelu(x):
    return jax.nn.gelu(x, approximate=True)
def _silu(x):
    return jax.nn.silu(x)
def _sigmoid(x):
    return jax.nn.sigmoid(x)
def _layernorm(x, axis=-1, eps=1e-5):
    m = jnp.mean(x, axis=axis, keepdims=True)
    v = jnp.var(x, axis=axis, keepdims=True)
    return (x - m) / jnp.sqrt(v + eps)
def _scatter_add(tgt, idx, src, axis=0):
    return tgt.at[idx].add(src)
def _segment_sum(src, seg, n):
    return jax.ops.segment_sum(src, seg, n)
class _Rng:
    def __init__(self, key):
        self._k = key
    def _next(self):
        self._k, sub = jax.random.split(self._k)
        return sub
    def normal(self, shape):
        return jax.random.normal(self._next(), shape, dtype=jnp.bfloat16)
    def randint(self, lo, hi, shape):
        return jax.random.randint(self._next(), shape, lo, hi, dtype=jnp.int32)
    def uniform(self, shape, lo=0.0, hi=1.0):
        return jax.random.uniform(self._next(), shape, jnp.bfloat16, lo, hi)
    def permutation(self, n):
        return jax.random.permutation(self._next(), n)


kernel_name = 'standalone__gqa_block_cached__near_ridge'

def setup_inputs():
    _rng = _Rng(jax.random.key(int.from_bytes(__import__("os").urandom(4), "little")))
    _w = (lambda a: (lambda t: t.astype(jnp.bfloat16) if jnp.issubdtype(t.dtype, jnp.floating) else t)(jnp.asarray(a)))
    B, Sq, D = 16, 128, 576
    Hq, Hkv, Sk, Dh = 32, 16, 1024, 128
    assert Hq % Hkv == 0, (Hq, Hkv)
    return {
        "x": _w((lambda *s: _rng.normal(s) * 0.8)(B, Sq, D)),
        "k_cache": _w((lambda *s: _rng.normal(s) * 0.8)(B, Hkv, Sk, Dh)),
        "v_cache": _w((lambda *s: _rng.normal(s) * 0.05)(B, Hkv, Sk, Dh)),
        "wq": _w((lambda *s: _rng.normal(s) * 0.8)(D, Hq * Dh) * (D ** -0.5)),
        "wo": _w((lambda *s: _rng.normal(s) * 0.05)(Hq * Dh, D) * ((Hq * Dh) ** -0.5)),
    }

def reference(x, k_cache, v_cache, wq, wo):
    B, Sq, D = x.shape
    Hq, Dh = 32, 128
    Hkv = k_cache.shape[1]
    rep = Hq // Hkv
    q = (lambda x, *d: x.transpose(*d))((x @ wq).reshape(B, Sq, Hq, Dh), 0, 2, 1, 3)
    k = jnp.repeat(k_cache, rep, axis=1)
    v = jnp.repeat(v_cache, rep, axis=1)
    scores = jnp.einsum("bhqd,bhkd->bhqk", q, k) * (Dh ** -0.5)
    p = _softmax(scores, axis=-1)
    o = jnp.einsum("bhqk,bhkd->bhqd", p, v)
    return (lambda x, *d: x.transpose(*d))(o, 0, 2, 1, 3).reshape(B, Sq, Hq * Dh) @ wo
```

```python
import jax
import jax.numpy as jnp
import numpy as np
import jax.experimental.pallas as pl
import jax.experimental.pallas.tpu as pltpu

LOG2E = 1.4426950408889634
NT = (((1,), (1,)), ((), ()))


def make(G=8, GR=2, seq="BACED", seq_r="BACED", vmem=100):
  def gqa_block(x, k_cache, v_cache, wq, wo):
    B, Sq, D = x.shape
    _, Hkv, Sk, Dh = k_cache.shape
    REP = wq.shape[1] // (Hkv * Dh)
    R = REP * Sq
    scale = (Dh ** -0.5) * LOG2E
    N = B * Hkv
    NG = N // G
    GPH = B // G
    NR = G // GR
    NK, NV = 2, 4
    DP = -(-D // 128) * 128
    assert B % G == 0 and G % GR == 0 and GR % 2 == 0 and G < B and NR >= 3 and Sq == 128 and Dh == 128
    bf, f32 = jnp.bfloat16, jnp.float32
    xT = x.transpose(0, 2, 1)
    woT = wo.T

    def kernel(xT_hbm, k_hbm, v_hbm, wq_hbm, woT_hbm, o_hbm,
               x_in, x_sc, wq_sc, wo_sc, k_buf, v_buf, acc_sc, out_sc,
               s0, s1, p0, p1, l0, l1, q_c, o_c,
               sem_x, sem_w, sem_k, sem_v, sem_kr, sem_vr, sem_o):
        s_b, p_b, l_b = (s0, s1), (p0, p1), (l0, l1)

        def x_copy(b):
            return pltpu.make_async_copy(xT_hbm.at[b], x_in.at[b], sem_x.at[b])
        def w_copies(h):
            cs = []
            for r in range(REP):
                col = pl.ds(pl.multiple_of((h * REP + r) * Dh, Dh), Dh)
                cs.append(pltpu.make_async_copy(wq_hbm.at[:, col], wq_sc.at[h * REP + r], sem_w.at[(h % 2) * 2 * REP + r]))
                cs.append(pltpu.make_async_copy(woT_hbm.at[:, col], wo_sc.at[h * REP + r], sem_w.at[(h % 2) * 2 * REP + REP + r]))
            return cs
        def k_copy(g, slot):
            return pltpu.make_async_copy(k_hbm.at[pl.ds((g % GPH) * G, G), g // GPH], k_buf.at[slot], sem_k.at[slot])
        def v_copy(g, slot):
            return pltpu.make_async_copy(v_hbm.at[pl.ds((g % GPH) * G, G), g // GPH], v_buf.at[slot], sem_v.at[slot])
        def kr_copy(r):
            return pltpu.make_async_copy(k_hbm.at[pl.ds(r * GR, GR), 0], k_buf.at[0, pl.ds(r * GR, GR)], sem_kr.at[r])
        def vr_copy(r):
            return pltpu.make_async_copy(v_hbm.at[pl.ds(r * GR, GR), 0], v_buf.at[0, pl.ds(r * GR, GR)], sem_vr.at[r])
        def out_copy(b):
            return pltpu.make_async_copy(out_sc.at[b], o_hbm.at[b], sem_o.at[b])
        def x_transpose(b):
            x_copy(b).wait()
            xt = x_in[b].astype(f32)
            xt = jnp.concatenate([xt, jnp.zeros((DP - D, Sq), f32)], axis=0)
            x_sc[b] = xt.T[:, :D].astype(bf)

        def q_proj(h, b):
            w = jnp.concatenate([wq_sc[h * REP + r] for r in range(REP)], axis=1)
            q = jnp.dot(x_sc[b], w, preferred_element_type=f32)
            q = (q * scale).astype(bf)
            return jnp.concatenate([q[:, r * Dh:(r + 1) * Dh] for r in range(REP)], axis=0)
        def scores(q, k_ref, par):
            s_b[par][...] = jax.lax.dot_general(q, k_ref[...], NT, preferred_element_type=f32)
        def softmax(par):
            m = jnp.max(s_b[par][...], axis=-1, keepdims=True)
            p = jnp.exp2(s_b[par][...] - m)
            l = jnp.sum(p, axis=-1, keepdims=True)
            r = pl.reciprocal(l, approx=True)
            r = r * (2.0 - l * r)
            p_b[par][...] = p.astype(bf)
            l_b[par][...] = jnp.broadcast_to(r, (R, Dh))
        def pv(v_ref, par):
            o = jnp.dot(p_b[par][...], v_ref[...], preferred_element_type=f32)
            o = (o * l_b[par][...]).astype(bf)
            return jnp.concatenate([o[r * Sq:(r + 1) * Sq] for r in range(REP)], axis=1)
        def o_proj(h, slot, o):
            w = jnp.concatenate([wo_sc[h * REP + r] for r in range(REP)], axis=1)
            acc_sc[slot] += jax.lax.dot_general(w, o, NT, preferred_element_type=f32)

        def block(n, order, h, b0, k_at, v_at, a_last, d_first):
            q = q_c[...]
            os_ = {}
            for i in range(n):
                par = i % 2
                qn = None
                for st in order:
                    if st == "A":
                        qn = q_proj(*a_last) if i == n - 1 else q_proj(h, b0 + i + 1)
                    elif st == "B":
                        scores(q, k_at(i), par)
                    elif st == "C":
                        softmax(par)
                    elif st == "E":
                        os_[i - 1] = pv(v_at(i - 1), 1 - par)
                    elif st == "D":
                        o = o_c[...] if i == 0 else os_[i - 2]
                        if i < 2:
                            o_proj(*d_first(i), o)
                        else:
                            o_proj(h, b0 + i - 2, o)
                q = qn
            q_c[...] = q
            o_c[...] = os_[n - 2]

        w0 = w_copies(0)
        x_copy(0).start()
        for c in w0: c.start()
        kr_copy(0).start()
        for b in range(1, GR + 1): x_copy(b).start()
        vr_copy(0).start()
        for b in range(GR + 1, 2 * GR + 1): x_copy(b).start()
        kr_copy(1).start(); vr_copy(1).start()
        for b in range(B + 1):
            acc_sc[b] = jnp.zeros((D, Sq), f32)
        p_b[1][...] = jnp.zeros((R, Sk), bf)
        l_b[1][...] = jnp.zeros((R, Dh), f32)
        o_c[...] = jnp.zeros((Sq, R), bf)
        v_buf[NV - 1, G - 1] = jnp.zeros((Sk, Dh), bf)
        x_transpose(0)
        for c in w0: c.wait()
        q_c[...] = q_proj(0, 0)

        def ramp(r, carry):
            b0 = r * GR
            @pl.when(r + 2 < NR)
            def _():
                for i in range(GR): x_copy(b0 + 2 * GR + 1 + i).start()
                kr_copy(r + 2).start(); vr_copy(r + 2).start()
            @pl.when(r == 0)
            def _(): k_copy(1, 1 % NK).start()
            @pl.when(r == 1)
            def _(): v_copy(1, 1 % NV).start()
            @pl.when(r == 2)
            def _():
                for b in range(G + 1, B): x_copy(b).start()
                for c in w_copies(1): c.start()
            for i in range(GR): x_transpose(b0 + i + 1)
            kr_copy(r).wait(); vr_copy(r).wait()
            first = r == 0
            prev = (jnp.where(first, NV - 1, 0), jnp.where(first, G - 1, jnp.maximum(b0 - 1, 0)))
            block(GR, seq_r, 0, b0,
                  lambda i: k_buf.at[0, b0 + i],
                  lambda i: v_buf.at[prev] if i < 0 else v_buf.at[0, b0 + i],
                  (0, b0 + GR),
                  lambda i: (0, jnp.where(b0 + i - 2 < 0, B, b0 + i - 2)))
            return carry
        jax.lax.fori_loop(0, NR, ramp, 0)

        def body(g, carry):
            h = g // GPH
            jb = g % GPH
            @pl.when(jb == GPH - 1)
            def _():
                @pl.when(h + 1 < Hkv)
                def _():
                    for c in w_copies(h + 1): c.wait()
                @pl.when(h + 2 < Hkv)
                def _():
                    for c in w_copies(h + 2): c.start()
            @pl.when(g < GPH)
            def _():
                for i in range(G):
                    @pl.when(g * G + i + 1 < B)
                    def _(): x_transpose(jnp.minimum(g * G + i + 1, B - 1))
            kslot, vslot, vprev = g % NK, g % NV, (g + NV - 1) % NV
            k_copy(g, kslot).wait()
            v_copy(g, vslot).wait()
            gn = jnp.where(g + 1 < NG, g + 1, 0)
            k_copy(gn, (g + 1) % NK).start()
            v_copy(gn, (g + 1) % NV).start()
            last_of_head = jb == GPH - 1
            a_last = (jnp.where(last_of_head, jnp.minimum(h + 1, Hkv - 1), h),
                      jnp.where(last_of_head, 0, (jb + 1) * G))
            h_prev = jnp.where(jb == 0, h - 1, h)
            block(G, seq, h, jb * G,
                  lambda i: k_buf.at[kslot, i],
                  lambda i: v_buf.at[vprev, G - 1] if i < 0 else v_buf.at[vslot, i],
                  a_last,
                  lambda i: (h_prev, (jb * G + i - 2 + B) % B))
            @pl.when(h == Hkv - 1)
            def _():
                for i in range(G):
                    @pl.when(jb * G + i - 2 >= 0)
                    def _():
                        b = jnp.maximum(jb * G + i - 2, 0)
                        out_sc[b] = acc_sc[b].astype(bf)
                        out_copy(b).start()
            return carry
        jax.lax.fori_loop(1, NG, body, 0)

        o_proj(Hkv - 1, B - 2, o_c[...])
        o_last = pv(v_buf.at[(NG - 1) % NV, G - 1], (N - 1) % 2)
        out_sc[B - 2] = acc_sc[B - 2].astype(bf)
        out_copy(B - 2).start()
        o_proj(Hkv - 1, B - 1, o_last)
        out_sc[B - 1] = acc_sc[B - 1].astype(bf)
        out_copy(B - 1).start()
        k_copy(0, NG % NK).wait()
        v_copy(0, NG % NV).wait()
        for b in range(B):
            out_copy(b).wait()

    hbm = pl.BlockSpec(memory_space=pl.ANY)
    dma = lambda n: pltpu.SemaphoreType.DMA((n,))
    outT = pl.pallas_call(
        kernel,
        in_specs=[hbm] * 5,
        out_specs=hbm,
        out_shape=jax.ShapeDtypeStruct((B, D, Sq), x.dtype),
        scratch_shapes=[
            pltpu.VMEM((B, D, Sq), bf),
            pltpu.VMEM((B, Sq, D), bf),
            pltpu.VMEM((Hkv * REP, D, Dh), bf),
            pltpu.VMEM((Hkv * REP, D, Dh), bf),
            pltpu.VMEM((NK, G, Sk, Dh), bf),
            pltpu.VMEM((NV, G, Sk, Dh), bf),
            pltpu.VMEM((B + 1, D, Sq), f32),
            pltpu.VMEM((B, D, Sq), bf),
            pltpu.VMEM((R, Sk), f32), pltpu.VMEM((R, Sk), f32),
            pltpu.VMEM((R, Sk), bf), pltpu.VMEM((R, Sk), bf),
            pltpu.VMEM((R, Dh), f32), pltpu.VMEM((R, Dh), f32),
            pltpu.VMEM((R, Dh), bf),
            pltpu.VMEM((Sq, R), bf),
            dma(B), dma(4 * REP), dma(NK), dma(NV), dma(NR), dma(NR), dma(B),
        ],
        compiler_params=pltpu.CompilerParams(vmem_limit_bytes=vmem * 1024 * 1024,
                                             disable_bounds_checks=True),
    )(xT, k_cache, v_cache, wq, woT)
    return outT.transpose(0, 2, 1)
  return gqa_block


pallas_standalone__gqa_block_cached__near_ridge_kernel = jax.jit(make())
```

```python
import jax
import jax.numpy as jnp
import numpy as np
import jax.experimental.pallas as pl
import jax.experimental.pallas.tpu as pltpu

LOG2E = 1.4426950408889634
NT = (((1,), (1,)), ((), ()))


def make(G=8, GR=2, seq="BACED", seq_r="ABCED", vmem=100):
  def gqa_block(x, k_cache, v_cache, wq, wo):
    B, Sq, D = x.shape
    _, Hkv, Sk, Dh = k_cache.shape
    REP = wq.shape[1] // (Hkv * Dh)
    R = REP * Sq
    scale = (Dh ** -0.5) * LOG2E
    N = B * Hkv
    NG = N // G
    GPH = B // G
    NR = B // GR
    G0 = B // G
    NK, NV = 2, 4
    DP = -(-D // 128) * 128
    assert B % G == 0 and G % GR == 0 and GR % 2 == 0 and G0 == 2 and Sq == 128 and Dh == 128
    bf, f32 = jnp.bfloat16, jnp.float32
    xT = x.transpose(0, 2, 1)
    woT = wo.T

    def kernel(xT_hbm, k_hbm, v_hbm, wq_hbm, woT_hbm, o_hbm,
               x_in, x_sc, wq_sc, wo_sc, k_buf, v_buf, acc_sc, out_sc,
               s0, s1, p0, p1, l0, l1, q_c, o_c,
               sem_x, sem_w, sem_k, sem_v, sem_kr, sem_vr, sem_o):
        s_b, p_b, l_b = (s0, s1), (p0, p1), (l0, l1)

        def x_copy(b):
            return pltpu.make_async_copy(xT_hbm.at[b], x_in.at[b], sem_x.at[b])
        def w_copies(h):
            cs = []
            for r in range(REP):
                col = pl.ds(pl.multiple_of((h * REP + r) * Dh, Dh), Dh)
                cs.append(pltpu.make_async_copy(wq_hbm.at[:, col], wq_sc.at[h * REP + r], sem_w.at[(h % 2) * 2 * REP + r]))
                cs.append(pltpu.make_async_copy(woT_hbm.at[:, col], wo_sc.at[h * REP + r], sem_w.at[(h % 2) * 2 * REP + REP + r]))
            return cs
        def k_copy(g, slot):
            return pltpu.make_async_copy(k_hbm.at[pl.ds((g % GPH) * G, G), g // GPH], k_buf.at[slot], sem_k.at[slot])
        def v_copy(g, slot):
            return pltpu.make_async_copy(v_hbm.at[pl.ds((g % GPH) * G, G), g // GPH], v_buf.at[slot], sem_v.at[slot])
        def kr_copy(r):
            return pltpu.make_async_copy(k_hbm.at[pl.ds(r * GR, GR), 0], k_buf.at[(r * GR) // G, pl.ds((r * GR) % G, GR)], sem_kr.at[r])
        def vr_copy(r):
            return pltpu.make_async_copy(v_hbm.at[pl.ds(r * GR, GR), 0], v_buf.at[(r * GR) // G, pl.ds((r * GR) % G, GR)], sem_vr.at[r])
        def out_copy(b):
            return pltpu.make_async_copy(out_sc.at[b], o_hbm.at[b], sem_o.at[b])
        def x_transpose(b):
            x_copy(b).wait()
            xt = x_in[b].astype(f32)
            xt = jnp.concatenate([xt, jnp.zeros((DP - D, Sq), f32)], axis=0)
            x_sc[b] = xt.T[:, :D].astype(bf)

        def q_proj(h, b):
            w = jnp.concatenate([wq_sc[h * REP + r] for r in range(REP)], axis=1)
            q = jnp.dot(x_sc[b], w, preferred_element_type=f32)
            q = (q * scale).astype(bf)
            return jnp.concatenate([q[:, r * Dh:(r + 1) * Dh] for r in range(REP)], axis=0)
        def scores(q, k_ref, par):
            s_b[par][...] = jax.lax.dot_general(q, k_ref[...], NT, preferred_element_type=f32)
        def softmax(par):
            m = jnp.max(s_b[par][...], axis=-1, keepdims=True)
            p = jnp.exp2(s_b[par][...] - m)
            l = jnp.sum(p, axis=-1, keepdims=True)
            r = pl.reciprocal(l, approx=True)
            r = r * (2.0 - l * r)
            p_b[par][...] = p.astype(bf)
            l_b[par][...] = jnp.broadcast_to(r, (R, Dh))
        def pv(v_ref, par):
            o = jnp.dot(p_b[par][...], v_ref[...], preferred_element_type=f32)
            o = (o * l_b[par][...]).astype(bf)
            return jnp.concatenate([o[r * Sq:(r + 1) * Sq] for r in range(REP)], axis=1)
        def o_proj(h, slot, o):
            w = jnp.concatenate([wo_sc[h * REP + r] for r in range(REP)], axis=1)
            acc_sc[slot] += jax.lax.dot_general(w, o, NT, preferred_element_type=f32)

        def block(n, order, h, b0, k_at, v_at, a_last, d_first, fill=False):
            q = q_c[...]
            os_ = {}
            for i in range(n):
                par = i % 2
                qn = None
                for st in order:
                    if st == "A":
                        qn = q_proj(*a_last) if i == n - 1 else q_proj(h, b0 + i + 1)
                    elif st == "B":
                        scores(q, k_at(i), par)
                    elif st == "C":
                        softmax(par)
                    elif st == "E":
                        if fill and i == 0: continue
                        os_[i - 1] = pv(v_at(i - 1), 1 - par)
                    elif st == "D":
                        if fill and i < 2: continue
                        o = o_c[...] if i == 0 else os_[i - 2]
                        if i < 2:
                            o_proj(*d_first(i), o)
                        else:
                            o_proj(h, b0 + i - 2, o)
                q = qn
            q_c[...] = q
            o_c[...] = os_[n - 2]

        w0 = w_copies(0)
        x_copy(0).start()
        for c in w0: c.start()
        kr_copy(0).start()
        for b in range(1, GR + 1): x_copy(b).start()
        vr_copy(0).start()
        for b in range(GR + 1, 2 * GR + 1): x_copy(b).start()
        kr_copy(1).start(); vr_copy(1).start()
        for b in range(B):
            acc_sc[b] = jnp.zeros((D, Sq), f32)
        x_transpose(0)
        for c in w0: c.wait()
        q_c[...] = q_proj(0, 0)

        def ramp(r, carry, fill=False):
            b0 = r * GR
            @pl.when(r + 2 < NR)
            def _():
                for i in range(GR):
                    @pl.when(b0 + 2 * GR + 1 + i < B)
                    def _(): x_copy(jnp.minimum(b0 + 2 * GR + 1 + i, B - 1)).start()
                kr_copy(r + 2).start(); vr_copy(r + 2).start()
            @pl.when(r == 0)
            def _(): v_copy(G0, G0 % NV).start()
            @pl.when(r == 1)
            def _():
                for c in w_copies(1): c.start()
            @pl.when(r == G // GR)
            def _(): k_copy(G0, G0 % NK).start()
            @pl.when(r == NR - 1)
            def _():
                for c in w_copies(1): c.wait()
                for c in w_copies(2): c.start()
            for i in range(GR):
                @pl.when(b0 + i + 1 < B)
                def _(): x_transpose(jnp.minimum(b0 + i + 1, B - 1))
            kr_copy(r).wait(); vr_copy(r).wait()
            slot, off = b0 // G, b0 % G
            block(GR, seq_r, 0, b0,
                  lambda i: k_buf.at[slot, off + i],
                  lambda i: v_buf.at[(b0 - 1) // G, (b0 - 1) % G] if i < 0 else v_buf.at[slot, off + i],
                  ((b0 + GR) // B, (b0 + GR) % B),
                  lambda i: (0, b0 + i - 2), fill)
            return carry
        ramp(0, 0, fill=True)
        jax.lax.fori_loop(1, NR, ramp, 0)

        def body(g, carry):
            h = g // GPH
            jb = g % GPH
            @pl.when(jb == GPH - 1)
            def _():
                @pl.when(h + 1 < Hkv)
                def _():
                    for c in w_copies(h + 1): c.wait()
                @pl.when(h + 2 < Hkv)
                def _():
                    for c in w_copies(h + 2): c.start()
            kslot, vslot, vprev = g % NK, g % NV, (g + NV - 1) % NV
            k_copy(g, kslot).wait()
            v_copy(g, vslot).wait()
            gn = jnp.where(g + 1 < NG, g + 1, 0)
            k_copy(gn, (g + 1) % NK).start()
            v_copy(gn, (g + 1) % NV).start()
            last_of_head = jb == GPH - 1
            a_last = (jnp.where(last_of_head, jnp.minimum(h + 1, Hkv - 1), h),
                      jnp.where(last_of_head, 0, (jb + 1) * G))
            h_prev = jnp.where(jb == 0, h - 1, h)
            block(G, seq, h, jb * G,
                  lambda i: k_buf.at[kslot, i],
                  lambda i: v_buf.at[vprev, G - 1] if i < 0 else v_buf.at[vslot, i],
                  a_last,
                  lambda i: (h_prev, (jb * G + i - 2 + B) % B))
            @pl.when(h == Hkv - 1)
            def _():
                for i in range(G):
                    @pl.when(jb * G + i - 2 >= 0)
                    def _():
                        b = jnp.maximum(jb * G + i - 2, 0)
                        out_sc[b] = acc_sc[b].astype(bf)
                        out_copy(b).start()
            return carry
        jax.lax.fori_loop(G0, NG, body, 0)

        o_proj(Hkv - 1, B - 2, o_c[...])
        o_last = pv(v_buf.at[(NG - 1) % NV, G - 1], (N - 1) % 2)
        out_sc[B - 2] = acc_sc[B - 2].astype(bf)
        out_copy(B - 2).start()
        o_proj(Hkv - 1, B - 1, o_last)
        out_sc[B - 1] = acc_sc[B - 1].astype(bf)
        out_copy(B - 1).start()
        k_copy(0, NG % NK).wait()
        v_copy(0, NG % NV).wait()
        for b in range(B):
            out_copy(b).wait()

    hbm = pl.BlockSpec(memory_space=pl.ANY)
    dma = lambda n: pltpu.SemaphoreType.DMA((n,))
    outT = pl.pallas_call(
        kernel,
        in_specs=[hbm] * 5,
        out_specs=hbm,
        out_shape=jax.ShapeDtypeStruct((B, D, Sq), x.dtype),
        scratch_shapes=[
            pltpu.VMEM((B, D, Sq), bf),
            pltpu.VMEM((B, Sq, D), bf),
            pltpu.VMEM((Hkv * REP, D, Dh), bf),
            pltpu.VMEM((Hkv * REP, D, Dh), bf),
            pltpu.VMEM((NK, G, Sk, Dh), bf),
            pltpu.VMEM((NV, G, Sk, Dh), bf),
            pltpu.VMEM((B, D, Sq), f32),
            pltpu.VMEM((B, D, Sq), bf),
            pltpu.VMEM((R, Sk), f32), pltpu.VMEM((R, Sk), f32),
            pltpu.VMEM((R, Sk), bf), pltpu.VMEM((R, Sk), bf),
            pltpu.VMEM((R, Dh), f32), pltpu.VMEM((R, Dh), f32),
            pltpu.VMEM((R, Dh), bf),
            pltpu.VMEM((Sq, R), bf),
            dma(B), dma(4 * REP), dma(NK), dma(NV), dma(NR), dma(NR), dma(B),
        ],
        compiler_params=pltpu.CompilerParams(vmem_limit_bytes=vmem * 1024 * 1024,
                                             disable_bounds_checks=True),
    )(xT, k_cache, v_cache, wq, woT)
    return outT.transpose(0, 2, 1)
  return gqa_block


pallas_standalone__gqa_block_cached__near_ridge_kernel = jax.jit(make())
```
